```python
import os as _os
_os.environ.setdefault("JAX_PLATFORMS", "cpu")
import jax
import jax.numpy as jnp

def _softmax(x, axis=-1):
    return jax.nn.softmax(x, axis=axis)
def _gelu(x):
    return jax.nn.gelu(x, approximate=True)
def _silu(x):
    return jax.nn.silu(x)
def _sigmoid(x):
    return jax.nn.sigmoid(x)
def _layernorm(x, axis=-1, eps=1e-5):
    m = jnp.mean(x, axis=axis, keepdims=True)
    v = jnp.var(x, axis=axis, keepdims=True)
    return (x - m) / jnp.sqrt(v + eps)
def _scatter_add(tgt, idx, src, axis=0):
    return tgt.at[idx].add(src)
def _segment_sum(src, seg, n):
    return jax.ops.segment_sum(src, seg, n)
class _Rng:
    def __init__(self, key):
        self._k = key
    def _next(self):
        self._k, sub = jax.random.split(self._k)
        return sub
    def normal(self, shape):
        return jax.random.normal(self._next(), shape, dtype=jnp.bfloat16)
    def randint(self, lo, hi, shape):
        return jax.random.randint(self._next(), shape, lo, hi, dtype=jnp.int32)
    def uniform(self, shape, lo=0.0, hi=1.0):
        return jax.random.uniform(self._next(), shape, jnp.bfloat16, lo, hi)
    def permutation(self, n):
        return jax.random.permutation(self._next(), n)


kernel_name = 'sequential_preLN__sliding_block__mixer_channel_mlp__prompt'

def setup_inputs():
    _rng = _Rng(jax.random.key(int.from_bytes(__import__("os").urandom(4), "little")))
    _w = (lambda a: (lambda t: t.astype(jnp.bfloat16) if jnp.issubdtype(t.dtype, jnp.floating) else t)(jnp.asarray(a)))
    def _A_setup():
        B, S, D = 1, 2048, 1024
        return {
            "x": _w((lambda *s: _rng.normal(s) * 0.05)(B, S, D)),
            "wqkv": _w((lambda *s: _rng.normal(s) * 0.05)(D, 3 * D)),
            "wo": _w((lambda *s: _rng.normal(s) * 0.05)(D, D)),
        }
    _A_in = _A_setup()

    def _B_setup():
        B, S, D, F = 1, 2048, 1024, 3584
        return {
            "x": _w((lambda *s: _rng.normal(s) * 0.05)(B, S, D)),
            "w1": _w((lambda *s: _rng.normal(s) * 0.8)(D, F) * (D ** -0.5)),
            "b1": _w((lambda *s: _rng.normal(s) * 0.8)(F)),
            "w2": _w((lambda *s: _rng.normal(s) * 0.8)(F, D) * (F ** -0.5)),
            "b2": _w((lambda *s: _rng.normal(s) * 0.05)(D)),
        }
    _B_in = _B_setup()

    return {
        "A_x": _A_in["x"],
        "A_wqkv": _A_in["wqkv"],
        "A_wo": _A_in["wo"],
        "B_x": _B_in["x"],
        "B_w1": _B_in["w1"],
        "B_b1": _B_in["b1"],
        "B_w2": _B_in["w2"],
        "B_b2": _B_in["b2"],
    }

def reference(A_x, A_wqkv, A_wo, B_x, B_w1, B_b1, B_w2, B_b2):
    def _A_ref(x, wqkv, wo):
        B, S, D = x.shape
        H = 32; Dh = D // H; W = 256
        qkv = (lambda x, *d: x.transpose(*d))((x @ wqkv).reshape(B, S, 3, H, Dh), 2, 0, 3, 1, 4)
        q, k, v = qkv[0], qkv[1], qkv[2]
        scores = jnp.einsum("bhqd,bhkd->bhqk", q, k) * (Dh ** -0.5)
        idx = jnp.arange(S)
        mask = (idx[:, None] - idx[None, :] >= 0) & (idx[:, None] - idx[None, :] < W)
        scores = jnp.where(mask[None, None], scores, -1e9)
        p = _softmax(scores, axis=-1)
        o = jnp.einsum("bhqk,bhkd->bhqd", p, v)
        return (lambda x, *d: x.transpose(*d))(o, 0, 2, 1, 3).reshape(B, S, D) @ wo

    def _B_ref(x, w1, b1, w2, b2):
        y = _layernorm(x, axis=-1)
        h = _gelu(jnp.einsum("bsd,df->bsf", y, w1) + b1)
        return jnp.einsum("bsf,fd->bsd", h, w2) + b2

    x = A_x
    h = x + _A_ref(_layernorm(x, axis=-1), A_wqkv, A_wo)
    h2 = h + _B_ref(_layernorm(h, axis=-1), B_w1, B_b1, B_w2, B_b2)
    return h2
```

```python
import functools
import jax
import jax.numpy as jnp
from jax import lax
import jax.experimental.pallas as pl
import jax.experimental.pallas.tpu as pltpu

S = 2048
D = 1024
F = 3584
H = 32
DH = 32
W = 256
T = 256
QT = 128
NQ = T // QT
NG = D // 128
EPS = 1e-5
NEG = -1e30
LOG2E = 1.4426950408889634
QSCALE = (DH ** -0.5) * LOG2E
GELU_C = 0.7978845608028654
BF = jnp.bfloat16
F32 = jnp.float32
NPART = 4
LNC = 16
PROWS = 3 * QT // NPART


def _ln(x):
    m = jnp.mean(x, axis=-1, keepdims=True)
    xc = x - m
    v = jnp.mean(xc * xc, axis=-1, keepdims=True)
    return xc * lax.rsqrt(v + EPS)


def _gelu(x):
    inner = x * (GELU_C + (GELU_C * 0.044715) * (x * x))
    return (0.5 * x) * (1.0 + jnp.tanh(inner))


def _dot(a, b):
    return jnp.dot(a, b, preferred_element_type=F32)


def _kernel(x_ref, xn_ref, wqkv_hbm, wo_hbm, w1_hbm, b1_ref, w2_hbm, b2_ref, o_ref,
            wqkv_v, wo_v, w1_v, w2_v, k_scr, vt_scr, y_scr, sems):
    i = pl.program_id(0)

    cp_qkv = pltpu.make_async_copy(wqkv_hbm, wqkv_v, sems.at[0])
    cp_wo = pltpu.make_async_copy(wo_hbm, wo_v, sems.at[1])
    cp_w1 = pltpu.make_async_copy(w1_hbm, w1_v, sems.at[2])
    cp_w2 = pltpu.make_async_copy(w2_hbm, w2_v, sems.at[3])

    @pl.when(i == 0)
    def _():
        cp_qkv.start()
        cp_wo.start()
        cp_w1.start()
        cp_w2.start()
        k_scr[0:W, :] = jnp.zeros((W, D), BF)
        vt_scr[0:W // QT] = jnp.zeros((W // QT, D, QT), BF)
        y_scr[...] = _ln(x_ref[...].astype(F32)).astype(BF)
        cp_qkv.wait()

    y = y_scr[...]
    qkv = _dot(y, wqkv_v[...])
    q = (qkv[:, :D] * QSCALE).astype(BF)
    k = qkv[:, D:2 * D].astype(BF)
    v = qkv[:, 2 * D:].astype(BF)
    row0 = pl.multiple_of(i * T, T)
    tbase = i * NQ
    k_scr[pl.ds(W + row0, T), :] = k
    qT = q.T
    vT = v.T
    for jj in range(NQ):
        vt_scr[W // QT + tbase + jj] = vT[:, jj * QT:(jj + 1) * QT]

    rr = lax.broadcasted_iota(jnp.int32, (QT, QT), 0)
    cc = lax.broadcasted_iota(jnp.int32, (QT, QT), 1)
    lo_mask = rr <= cc

    def qk_operands(u):
        j, g = divmod(u, NG)
        tile0 = tbase + j
        start = pl.multiple_of(tile0 * QT, QT)
        kwin = k_scr[pl.ds(start, 3 * QT), g * 128:(g + 1) * 128]
        parts = []
        for b in range(QT // 16):
            parts.append(kwin[16 * b:16 * b + 16])
            parts.append(kwin[2 * QT + 16 * b:2 * QT + 16 * b + 16])
        parts.append(kwin[QT:2 * QT])
        klhs = jnp.concatenate(parts, axis=0)
        ws = []
        for h in range(4):
            blk = qT[g * 128 + h * DH:g * 128 + (h + 1) * DH, j * QT:(j + 1) * QT]
            pieces = []
            if h > 0:
                pieces.append(jnp.zeros((h * DH, QT), BF))
            pieces.append(blk)
            if h < 3:
                pieces.append(jnp.zeros(((3 - h) * DH, QT), BF))
            ws.append(jnp.concatenate(pieces, axis=0))
        rhs = jnp.concatenate(ws, axis=1)
        return klhs, rhs

    def qk_part(ops, p):
        klhs, rhs = ops
        return _dot(klhs[p * PROWS:(p + 1) * PROWS], rhs)

    def softmax_pv(u, sT, h):
        j, g = divmod(u, NG)
        tile0 = tbase + j
        hb = jnp.where(tile0 >= 2, 0.0, NEG).astype(F32)
        mb = jnp.where(tile0 >= 1, 0.0, NEG).astype(F32)
        sh = sT[:, h * QT:(h + 1) * QT]
        s_hi = jnp.concatenate([sh[32 * b:32 * b + 16] for b in range(QT // 16)], axis=0)
        s_lo = jnp.concatenate([sh[32 * b + 16:32 * b + 32] for b in range(QT // 16)], axis=0)
        s_mid = sh[2 * QT:3 * QT]
        sm = jnp.where(lo_mask, s_lo, s_hi + hb)
        m = jnp.maximum(jnp.max(sm, axis=0, keepdims=True), jnp.max(s_mid, axis=0, keepdims=True) + mb)
        e_m = jnp.exp2(sm - m)
        e_mid = jnp.exp2(s_mid - (m - mb))
        l = jnp.sum(e_m + e_mid, axis=0, keepdims=True)
        p_lo = jnp.where(lo_mask, e_m, 0.0).astype(BF)
        p_hi = jnp.where(lo_mask, 0.0, e_m).astype(BF)
        r0 = g * 128 + h * DH
        acc = _dot(vt_scr[tile0, r0:r0 + DH, :], p_hi)
        acc += _dot(vt_scr[tile0 + 1, r0:r0 + DH, :], e_mid.astype(BF))
        acc += _dot(vt_scr[tile0 + 2, r0:r0 + DH, :], p_lo)
        return (acc * pl.reciprocal(l, approx=False)).astype(BF)

    NU = NQ * NG
    LAG = 1
    s_all = {}
    head_out = {}
    ops = qk_operands(0)
    s_all[0] = jnp.concatenate([qk_part(ops, p) for p in range(NPART)], axis=0)
    nxt = []
    for t in range(NU * 4 + LAG):
        un, p = divmod(t, 4)
        un += 1
        if un < NU:
            if p == 0:
                ops = qk_operands(un)
                nxt = []
            nxt.append(qk_part(ops, p))
            if p == NPART - 1:
                s_all[un] = jnp.concatenate(nxt, axis=0)
        hu = t - LAG
        if hu >= 0:
            u, h = divmod(hu, 4)
            head_out[hu] = softmax_pv(u, s_all[u], h)
    outs = [jnp.concatenate([head_out[4 * u + h] for h in range(4)], axis=0) for u in range(NU)]

    @pl.when(i == 0)
    def _():
        cp_wo.wait()
        cp_w1.wait()

    for c in range(T // LNC):
        y_scr[c * LNC:(c + 1) * LNC, :] = _ln(xn_ref[c * LNC:(c + 1) * LNC, :].astype(F32)).astype(BF)

    hres = []
    y2 = []
    for j in range(NQ):
        oT = jnp.concatenate(outs[j * NG:(j + 1) * NG], axis=0)
        o = oT.T
        attn = _dot(o, wo_v[...])
        ys = []
        for c in range(QT // LNC):
            r0 = j * QT + c * LNC
            hj = x_ref[r0:r0 + LNC, :].astype(F32) + attn[c * LNC:(c + 1) * LNC]
            hres.append(hj)
            ys.append(_ln(_ln(hj)).astype(BF))
        y2.append(jnp.concatenate(ys, axis=0))

    b1 = b1_ref[...].astype(F32)
    h1 = []
    for j in range(NQ):
        t = _dot(y2[j], w1_v[...]) + b1
        h1.append(_gelu(t).astype(BF))
    h1 = jnp.concatenate(h1, axis=0)

    @pl.when(i == 0)
    def _():
        cp_w2.wait()

    out = _dot(h1, w2_v[...])
    hr = jnp.concatenate(hres, axis=0)
    o_ref[...] = (hr + out + b2_ref[...].astype(F32)).astype(o_ref.dtype)


@jax.jit
def pallas_sequential_preLN__sliding_block__mixer_channel_mlp__prompt_kernel(A_x, A_wqkv, A_wo, B_x, B_w1, B_b1, B_w2, B_b2):
    x = A_x.reshape(S, D)
    b1 = B_b1.reshape(1, F)
    b2 = B_b2.reshape(1, D)
    nsteps = S // T
    out = pl.pallas_call(
        _kernel,
        grid=(nsteps,),
        in_specs=[
            pl.BlockSpec((T, D), lambda i: (i, 0)),
            pl.BlockSpec((T, D), lambda i: (jnp.minimum(i + 1, nsteps - 1), 0)),
            pl.BlockSpec(memory_space=pl.ANY),
            pl.BlockSpec(memory_space=pl.ANY),
            pl.BlockSpec(memory_space=pl.ANY),
            pl.BlockSpec((1, F), lambda i: (0, 0)),
            pl.BlockSpec(memory_space=pl.ANY),
            pl.BlockSpec((1, D), lambda i: (0, 0)),
        ],
        out_specs=pl.BlockSpec((T, D), lambda i: (i, 0)),
        out_shape=jax.ShapeDtypeStruct((S, D), BF),
        scratch_shapes=[
            pltpu.VMEM((D, 3 * D), BF),
            pltpu.VMEM((D, D), BF),
            pltpu.VMEM((D, F), BF),
            pltpu.VMEM((F, D), BF),
            pltpu.VMEM((W + S, D), BF),
            pltpu.VMEM((W // QT + S // QT, D, QT), BF),
            pltpu.VMEM((T, D), BF),
            pltpu.SemaphoreType.DMA((4,)),
        ],
        compiler_params=pltpu.CompilerParams(
            dimension_semantics=("arbitrary",),
            vmem_limit_bytes=100 * 1024 * 1024,
        ),
    )(x, x, A_wqkv, A_wo, B_w1, b1, B_w2, b2)
    return out.reshape(1, S, D)
```

```python
import functools
import jax
import jax.numpy as jnp
from jax import lax
import jax.experimental.pallas as pl
import jax.experimental.pallas.tpu as pltpu

S = 2048
D = 1024
F = 3584
H = 32
DH = 32
T = 256
QT = 128
HQ = 64
NQ = T // QT
NSTEPS = S // T
NG = D // 128
EPS = 1e-5
NEG = -1e30
LOG2E = 1.4426950408889634
QSCALE = (DH ** -0.5) * LOG2E
GELU_C = 0.7978845608028654
BF = jnp.bfloat16
F32 = jnp.float32
NPART = 4
LNC = 16
KROWS = 5 * HQ
PROWS = KROWS // NPART
WOC = 256
LAG = 1
WC = 512
NQKV = 3 * D // WC
NFC = F // WC
SEM_WO = NQKV
SEM_W1 = NQKV + 1
SEM_W2 = SEM_W1 + NFC
SEM_X = SEM_W2 + NFC
NSEM = SEM_X + S // T
G0 = 2


def _ln(x):
    m = jnp.mean(x, axis=-1, keepdims=True)
    xc = x - m
    v = jnp.mean(xc * xc, axis=-1, keepdims=True)
    return xc * lax.rsqrt(v + EPS)


def _gelu(x):
    inner = x * (GELU_C + (GELU_C * 0.044715) * (x * x))
    return (0.5 * x) * (1.0 + jnp.tanh(inner))


def _dot(a, b):
    return jnp.dot(a, b, preferred_element_type=F32)


def _pk(x):
    n = x.shape[0] // 16
    a = jnp.concatenate([x[16 * b:16 * b + 8] for b in range(n)], axis=0)
    b = jnp.concatenate([x[16 * b + 8:16 * b + 16] for b in range(n)], axis=0)
    return pltpu.pack_elementwise([a, b], packed_dtype=BF)


def _bf(x):
    return pltpu.bitcast(x, BF)


def _red8(x, op):
    parts = [x[8 * r:8 * r + 8] for r in range(x.shape[0] // 8)]
    while len(parts) > 1:
        parts = [op(parts[2 * r], parts[2 * r + 1]) for r in range(len(parts) // 2)] + (
            [parts[-1]] if len(parts) % 2 else [])
    return parts[0]


def _ln1_to(y_scr, x_v, row0):
    for c in range(T // LNC):
        x = x_v[pl.ds(row0 + c * LNC, LNC), :]
        y_scr[c * LNC:(c + 1) * LNC, :] = _ln(x.astype(F32)).astype(BF)


def _cp_x(x_hbm, x_v, sems, blk):
    rows = pl.ds(blk * T if isinstance(blk, int) else pl.multiple_of(blk * T, T), T)
    return pltpu.make_async_copy(x_hbm.at[rows, :], x_v.at[rows, :], sems.at[SEM_X + blk])


def _head_rhs(qT_blk):
    ws = []
    for h in range(4):
        pieces = []
        if h > 0:
            pieces.append(jnp.zeros((h * DH, QT), BF))
        pieces.append(qT_blk[h * DH:(h + 1) * DH])
        if h < 3:
            pieces.append(jnp.zeros(((3 - h) * DH, QT), BF))
        ws.append(jnp.concatenate(pieces, axis=0))
    return jnp.concatenate(ws, axis=1)


def _first_step(x_hbm, wqkv_hbm, wo_hbm, w1_hbm, b1_ref, w2_hbm, b2_ref, o_ref,
                x_v, wqkv_v, wo_v, w1_v, w2_v, k_scr, vt_scr, y_scr, raw_scr, qt_scr, ot_scr, acc_scr, sems):
    def col(c):
        return pl.ds(pl.multiple_of(c * WC, WC), WC)

    def cp_qkv(c):
        return pltpu.make_async_copy(wqkv_hbm.at[:, col(c)], wqkv_v.at[:, col(c)], sems.at[c])

    def cp_w1(c):
        return pltpu.make_async_copy(w1_hbm.at[:, col(c)], w1_v.at[:, col(c)], sems.at[SEM_W1 + c])

    def cp_w2(c):
        return pltpu.make_async_copy(w2_hbm.at[col(c), :], w2_v.at[col(c), :], sems.at[SEM_W2 + c])

    cp_wo = pltpu.make_async_copy(wo_hbm, wo_v, sems.at[SEM_WO])
    _cp_x(x_hbm, x_v, sems, 0).start()
    for c in range(NQKV):
        cp_qkv(c).start()
    _cp_x(x_hbm, x_v, sems, 1).start()
    cp_wo.start()
    for c in range(NFC):
        cp_w1(c).start()
        cp_w2(c).start()
    for blk in range(2, NSTEPS):
        _cp_x(x_hbm, x_v, sems, blk).start()

    _cp_x(x_hbm, x_v, sems, 0).wait()
    _ln1_to(y_scr, x_v, 0)

    def qkv_body(c, carry):
        cp_qkv(c).wait()
        scale = jnp.where(c < D // WC, QSCALE, 1.0).astype(F32)
        raw_scr[:, col(c)] = (_dot(y_scr[...], wqkv_v[:, col(c)]) * scale).astype(BF)
        return carry

    lax.fori_loop(0, NQKV, qkv_body, 0)

    qt_scr[...] = raw_scr[:, 0:D].T
    vT = _bf(_pk(raw_scr[:, 2 * D:3 * D].astype(F32))).T
    for jj in range(NQ):
        vt_scr[jj] = vT[:, jj * QT:(jj + 1) * QT]

    rr = lax.broadcasted_iota(jnp.int32, (QT, QT), 0)
    cc = lax.broadcasted_iota(jnp.int32, (QT, QT), 1)
    causal = rr <= cc

    def attn_scores(g):
        qT = qt_scr[pl.ds(pl.multiple_of(g * 128, 128), 128), :]
        kg = raw_scr[:, pl.ds(pl.multiple_of(D + g * 128, 128), 128)]
        return [_dot(kg[0:(j + 1) * QT], _head_rhs(qT[:, j * QT:(j + 1) * QT])) for j in range(NQ)]

    def attn_finish(g, scores):
        for j in range(NQ):
            for h in range(4):
                s = scores[j][:, h * QT:(h + 1) * QT]
                tiles = [s[t * QT:(t + 1) * QT] for t in range(j)] + [jnp.where(causal, s[j * QT:(j + 1) * QT], NEG)]
                m8 = _red8(tiles[0], jnp.maximum)
                for t in tiles[1:]:
                    m8 = jnp.maximum(m8, _red8(t, jnp.maximum))
                m = jnp.max(m8, axis=0, keepdims=True)
                es = [jnp.exp2(t - m) for t in tiles]
                l8 = _red8(es[0], jnp.add)
                for e in es[1:]:
                    l8 = l8 + _red8(e, jnp.add)
                l = jnp.sum(l8, axis=0, keepdims=True)
                rows = pl.ds(pl.multiple_of(g * 128 + h * DH, DH), DH)
                acc = _dot(vt_scr[0, rows, :], _bf(_pk(es[0])))
                for t in range(1, j + 1):
                    acc += _dot(vt_scr[t, rows, :], _bf(_pk(es[t])))
                ot_scr[rows, j * QT:(j + 1) * QT] = (acc * pl.reciprocal(l, approx=False)).astype(BF)

    def attn_body(gg, carry):
        scores = [attn_scores(gg * G0 + k) for k in range(G0)]
        for k in range(G0):
            attn_finish(gg * G0 + k, scores[k])
        return carry

    lax.fori_loop(0, NG // G0, attn_body, 0)

    cp_wo.wait()
    _cp_x(x_hbm, x_v, sems, 1).wait()
    k_scr[0:T, :] = raw_scr[:, D:2 * D]
    b2 = b2_ref[...].astype(F32).reshape(1, D)
    for j in range(NQ):
        attn = _dot(ot_scr[:, j * QT:(j + 1) * QT].T, wo_v[...])
        for c in range(QT // LNC):
            rows = slice(j * QT + c * LNC, j * QT + (c + 1) * LNC)
            hj = x_v[rows, :].astype(F32) + attn[c * LNC:(c + 1) * LNC]
            acc_scr[rows, :] = hj + b2
            raw_scr[rows, 0:D] = _ln(_ln(hj)).astype(BF)
    _ln1_to(y_scr, x_v, T)

    def mlp_body(c, carry):
        cp_w1(c).wait()
        cp_w2(c).wait()
        b1 = b1_ref[col(c)].astype(F32).reshape(1, WC)
        h = _gelu(_dot(raw_scr[:, 0:D], w1_v[:, col(c)]) + b1).astype(BF)
        acc_scr[...] += _dot(h, w2_v[col(c), :])
        return carry

    lax.fori_loop(0, NFC, mlp_body, 0)
    o_ref[...] = acc_scr[...].astype(o_ref.dtype)


def _main_step(i, b1_ref, b2_ref, o_ref, x_v, wqkv_v, wo_v, w1_v, w2_v, k_scr, vt_scr, y_scr):
    row0 = pl.multiple_of(i * T, T)
    rown = pl.multiple_of(jnp.minimum(i + 1, NSTEPS - 1) * T, T)
    qkv = _dot(y_scr[...], wqkv_v[...])
    q32 = qkv[:, :D] * QSCALE
    k = qkv[:, D:2 * D].astype(BF)
    v = _bf(_pk(qkv[:, 2 * D:]))
    tbase = i * NQ
    k_scr[pl.ds(row0, T), :] = k
    even_d = (lax.broadcasted_iota(jnp.int32, (HQ, D), 1) // DH) % 2 == 0
    ra, rb = [], []
    for j in range(NQ):
        qa = q32[j * QT:j * QT + HQ]
        qb = q32[j * QT + HQ:(j + 1) * QT]
        ra.append(jnp.concatenate([jnp.where(even_d, qa, 0.0), jnp.where(even_d, 0.0, qa)], axis=0).astype(BF).T)
        rb.append(jnp.concatenate([jnp.where(even_d, 0.0, qb), jnp.where(even_d, qb, 0.0)], axis=0).astype(BF).T)
    vT = v.T
    for jj in range(NQ):
        vt_scr[tbase + jj] = vT[:, jj * QT:(jj + 1) * QT]

    rr = lax.broadcasted_iota(jnp.int32, (HQ, QT), 0)
    cc = lax.broadcasted_iota(jnp.int32, (HQ, QT), 1)
    lo64 = rr <= (cc % HQ)
    left1 = lax.broadcasted_iota(jnp.int32, (1, QT), 1) < HQ
    pr = lax.broadcasted_iota(jnp.int32, (HQ // 2, QT), 0)
    pc = lax.broadcasted_iota(jnp.int32, (HQ // 2, QT), 1)
    ca = (pr // 8) * 16 + pr % 8
    lo_bits = (jnp.where(ca <= pc % HQ, jnp.uint32(0x0000FFFF), jnp.uint32(0))
               | jnp.where(ca + 8 <= pc % HQ, jnp.uint32(0xFFFF0000), jnp.uint32(0)))
    hi_bits = ~lo_bits
    pleft = pc < HQ
    zero_u = jnp.zeros((HQ // 2, QT), jnp.uint32)
    left_hi = jnp.where(pleft, hi_bits, zero_u)
    left_lo = jnp.where(pleft, lo_bits, zero_u)
    right_hi = jnp.where(pleft, zero_u, hi_bits)
    right_lo = jnp.where(pleft, zero_u, lo_bits)
    pleft2 = lax.broadcasted_iota(jnp.int32, (HQ, QT), 1) < HQ

    def interleave(hi, lo):
        parts = []
        for b in range(HQ // 16):
            parts.append(hi[16 * b:16 * b + 16])
            parts.append(lo[16 * b:16 * b + 16])
        return parts

    def qk_operands(u):
        j, g = divmod(u, NG)
        start = pl.multiple_of((tbase + j - 2) * QT, QT)
        kwin = k_scr[pl.ds(start, 3 * QT), g * 128:(g + 1) * 128]
        blk = [kwin[HQ * b:HQ * (b + 1)] for b in range(6)]
        lhs_a = jnp.concatenate(interleave(blk[0], blk[4]) + [blk[1], blk[2], blk[3]], axis=0)
        lhs_b = jnp.concatenate(interleave(blk[1], blk[5]) + [blk[2], blk[3], blk[4]], axis=0)
        rhs = []
        for r in (ra[j], rb[j]):
            tiles = []
            for p in range(2):
                rows = r[g * 128 + 64 * p:g * 128 + 64 * (p + 1), :]
                z = jnp.zeros((64, QT), BF)
                tiles.append(jnp.concatenate([rows, z] if p == 0 else [z, rows], axis=0))
            rhs.append(jnp.concatenate(tiles, axis=1))
        return lhs_a, lhs_b, rhs[0], rhs[1]

    def qk_part(ops, p):
        lhs_a, lhs_b, rhs_a, rhs_b = ops
        sl = slice(p * PROWS, (p + 1) * PROWS)
        return _dot(lhs_a[sl], rhs_a), _dot(lhs_b[sl], rhs_b)

    def deinterleave(s):
        hi = jnp.concatenate([s[32 * b:32 * b + 16] for b in range(HQ // 16)], axis=0)
        lo = jnp.concatenate([s[32 * b + 16:32 * b + 32] for b in range(HQ // 16)], axis=0)
        return hi, lo

    def stage0(u, s_pair, p):
        j, g = divmod(u, NG)
        t0 = tbase + j - 2
        sa = s_pair[0][:, p * QT:(p + 1) * QT]
        sb = s_pair[1][:, p * QT:(p + 1) * QT]
        jg = tbase + j
        b2 = jnp.where(jg >= 2, 0.0, NEG).astype(F32)
        b1 = jnp.where(jg >= 1, 0.0, NEG).astype(F32)
        hi, lo = deinterleave(sa[0:2 * HQ])
        ma = jnp.where(lo64, lo, hi + b2)
        a3, a21 = sa[2 * HQ:3 * HQ], sa[3 * HQ:5 * HQ]
        m_a = jnp.max(jnp.maximum(jnp.maximum(_red8(ma, jnp.maximum), _red8(a3, jnp.maximum) + b2),
                                  _red8(a21, jnp.maximum) + b1), axis=0, keepdims=True)
        hi, lo = deinterleave(sb[0:2 * HQ])
        mb = jnp.where(lo64, lo, hi + b2)
        b21, b0 = sb[2 * HQ:4 * HQ], sb[4 * HQ:5 * HQ]
        m_b = jnp.max(jnp.maximum(jnp.maximum(_red8(mb, jnp.maximum), _red8(b0, jnp.maximum)),
                                  _red8(b21, jnp.maximum) + b1), axis=0, keepdims=True)
        e_a21 = jnp.exp2(a21 - (m_a - b1))
        e_b21 = jnp.exp2(b21 - (m_b - b1))
        l_a = _red8(e_a21, jnp.add)
        l_b = _red8(e_b21, jnp.add)
        r0 = g * 128 + 2 * p * DH
        pa, pb = _pk(e_a21), _pk(e_b21)
        acc_e = _dot(vt_scr[t0 + 1, r0:r0 + DH, :], _bf(jnp.where(pleft2, pa, pb)))
        acc_o = _dot(vt_scr[t0 + 1, r0 + DH:r0 + 2 * DH, :], _bf(jnp.where(pleft2, pb, pa)))
        return (ma, a3, m_a, l_a), (mb, b0, m_b, l_b), acc_e, acc_o

    def stage1(u, p, st):
        j, g = divmod(u, NG)
        t0 = tbase + j - 2
        (ma, a3, m_a, l_a), (mb, b0, m_b, l_b), acc_e, acc_o = st
        e_ma = jnp.exp2(ma - m_a)
        e_a3 = jnp.exp2(a3 - m_a)
        e_mb = jnp.exp2(mb - m_b)
        e_b0 = jnp.exp2(b0 - m_b)
        l_a = jnp.sum(l_a + _red8(e_ma + e_a3, jnp.add), axis=0, keepdims=True)
        l_b = jnp.sum(l_b + _red8(e_mb + e_b0, jnp.add), axis=0, keepdims=True)
        pma, pa3, pmb, pb0 = _pk(e_ma), _pk(e_a3), _pk(e_mb), _pk(e_b0)
        ma_lo = pma & lo_bits
        mb_hi = pmb & hi_bits
        r0 = g * 128 + 2 * p * DH
        pe0 = jnp.concatenate([pma & left_hi, jnp.where(pleft, pa3, mb_hi)], axis=0)
        pe2 = jnp.concatenate([jnp.where(pleft, ma_lo, pb0), pmb & right_lo], axis=0)
        po0 = jnp.concatenate([pma & right_hi, jnp.where(pleft, mb_hi, pa3)], axis=0)
        po2 = jnp.concatenate([jnp.where(pleft, pb0, ma_lo), pmb & left_lo], axis=0)
        acc_e += _dot(vt_scr[t0, r0:r0 + DH, :], _bf(pe0))
        acc_o += _dot(vt_scr[t0, r0 + DH:r0 + 2 * DH, :], _bf(po0))
        acc_e += _dot(vt_scr[t0 + 2, r0:r0 + DH, :], _bf(pe2))
        acc_o += _dot(vt_scr[t0 + 2, r0 + DH:r0 + 2 * DH, :], _bf(po2))
        r_a = pl.reciprocal(l_a, approx=False)
        r_b = pl.reciprocal(l_b, approx=False)
        o_e = acc_e * jnp.where(left1, r_a, r_b)
        o_o = pltpu.roll(acc_o * jnp.where(left1, r_b, r_a), HQ, 1)
        return o_e.astype(BF), o_o.astype(BF)

    NU = NQ * NG
    s_all = {}
    pair_p = {}
    head_out = {}

    def o_tile(j):
        oT = jnp.concatenate([head_out[4 * u + h] for u in range(j * NG, (j + 1) * NG) for h in range(4)], axis=0)
        return oT.T

    def gather(parts):
        return (jnp.concatenate([x[0] for x in parts], axis=0), jnp.concatenate([x[1] for x in parts], axis=0))

    ops = qk_operands(0)
    s_all[0] = gather([qk_part(ops, p) for p in range(NPART)])
    nxt = []
    attn0 = []
    o0 = None
    for t in range(NU * 4 + LAG):
        un, p = divmod(t, 4)
        un += 1
        if un < NU:
            if p == 0:
                ops = qk_operands(un)
                nxt = []
            nxt.append(qk_part(ops, p))
            if p == NPART - 1:
                s_all[un] = gather(nxt)
                if un == NU - 1:
                    o0 = o_tile(0)
        if o0 is not None and len(attn0) < D // WOC:
            c = len(attn0)
            attn0.append(_dot(o0, wo_v[:, c * WOC:(c + 1) * WOC]))
        hu = t - LAG
        if hu >= 0:
            u, h = divmod(hu, 4)
            if h % 2 == 0:
                pair_p[u] = stage0(u, s_all[u], h // 2)
            else:
                head_out[hu - 1], head_out[hu] = stage1(u, h // 2, pair_p[u])
    while len(attn0) < D // WOC:
        c = len(attn0)
        attn0.append(_dot(o0, wo_v[:, c * WOC:(c + 1) * WOC]))
    attn0 = jnp.concatenate(attn0, axis=1)

    hres = []
    y2 = []
    for j in range(NQ):
        attn = attn0 if j == 0 else _dot(o_tile(j), wo_v[...])
        ys = []
        for c in range(QT // LNC):
            r0 = j * QT + c * LNC
            hj = x_v[pl.ds(row0 + r0, LNC), :].astype(F32) + attn[c * LNC:(c + 1) * LNC]
            hres.append(hj)
            ys.append(_ln(_ln(hj)).astype(BF))
        y2.append(jnp.concatenate(ys, axis=0))

    b1 = b1_ref[...].astype(F32).reshape(1, F)
    h1 = jnp.concatenate([_gelu(_dot(y2[j], w1_v[...]) + b1).astype(BF) for j in range(NQ)], axis=0)
    _ln1_to(y_scr, x_v, rown)
    out = _dot(h1, w2_v[...])
    hr = jnp.concatenate(hres, axis=0)
    o_ref[...] = (hr + out + b2_ref[...].astype(F32).reshape(1, D)).astype(o_ref.dtype)


def _kernel(x_hbm, wqkv_hbm, wo_hbm, w1_hbm, b1_ref, w2_hbm, b2_ref, o_ref,
            x_v, wqkv_v, wo_v, w1_v, w2_v, k_scr, vt_scr, y_scr, raw_scr, qt_scr, ot_scr, acc_scr, sems):
    i = pl.program_id(0)

    @pl.when(i == 0)
    def _():
        _first_step(x_hbm, wqkv_hbm, wo_hbm, w1_hbm, b1_ref, w2_hbm, b2_ref, o_ref,
                    x_v, wqkv_v, wo_v, w1_v, w2_v, k_scr, vt_scr, y_scr, raw_scr, qt_scr, ot_scr, acc_scr, sems)

    @pl.when(jnp.logical_and(i > 0, i + 1 < NSTEPS))
    def _():
        _cp_x(x_hbm, x_v, sems, i + 1).wait()

    @pl.when(i > 0)
    def _():
        _main_step(i, b1_ref, b2_ref, o_ref, x_v, wqkv_v, wo_v, w1_v, w2_v, k_scr, vt_scr, y_scr)


@jax.jit
def pallas_sequential_preLN__sliding_block__mixer_channel_mlp__prompt_kernel(A_x, A_wqkv, A_wo, B_x, B_w1, B_b1, B_w2, B_b2):
    x = A_x.reshape(S, D)
    out = pl.pallas_call(
        _kernel,
        grid=(NSTEPS,),
        in_specs=[
            pl.BlockSpec(memory_space=pl.ANY),
            pl.BlockSpec(memory_space=pl.ANY),
            pl.BlockSpec(memory_space=pl.ANY),
            pl.BlockSpec(memory_space=pl.ANY),
            pl.BlockSpec((F,), lambda i: (0,)),
            pl.BlockSpec(memory_space=pl.ANY),
            pl.BlockSpec((D,), lambda i: (0,)),
        ],
        out_specs=pl.BlockSpec((T, D), lambda i: (i, 0)),
        out_shape=jax.ShapeDtypeStruct((S, D), BF),
        scratch_shapes=[
            pltpu.VMEM((S, D), BF),
            pltpu.VMEM((D, 3 * D), BF),
            pltpu.VMEM((D, D), BF),
            pltpu.VMEM((D, F), BF),
            pltpu.VMEM((F, D), BF),
            pltpu.VMEM((S, D), BF),
            pltpu.VMEM((S // QT, D, QT), BF),
            pltpu.VMEM((T, D), BF),
            pltpu.VMEM((T, 3 * D), BF),
            pltpu.VMEM((D, T), BF),
            pltpu.VMEM((D, T), BF),
            pltpu.VMEM((T, D), F32),
            pltpu.SemaphoreType.DMA((NSEM,)),
        ],
        compiler_params=pltpu.CompilerParams(
            dimension_semantics=("arbitrary",),
            vmem_limit_bytes=100 * 1024 * 1024,
        ),
    )(x, A_wqkv, A_wo, B_w1, B_b1, B_w2, B_b2)
    return out.reshape(1, S, D)
```

```python
import jax
import jax.numpy as jnp
from jax import lax
import jax.experimental.pallas as pl
import jax.experimental.pallas.tpu as pltpu

S = 2048
D = 1024
F = 3584
DH = 32
T = 256
QT = 128
HQ = 64
NQ = T // QT
NSTEPS = S // T
NG = D // 128
EPS = 1e-5
NEG = -1e30
LOG2E = 1.4426950408889634
QSCALE = (DH ** -0.5) * LOG2E
GELU_C = 0.7978845608028654
BF = jnp.bfloat16
F32 = jnp.float32
NPART = 4
LNC = 16
KROWS = 5 * HQ
PROWS = KROWS // NPART
WOC = 128
LAGF = 1.75
YR = 128
FC0 = 512
WC = 512
NQKV = 3 * D // WC
NFC = F // WC
SEM_WO = NQKV
SEM_W1 = NQKV + 1
SEM_W2 = SEM_W1 + NFC
SEM_X = SEM_W2 + NFC
NSEM = SEM_X + S // T
G0 = 2


def _ln(x):
    m = jnp.mean(x, axis=-1, keepdims=True)
    xc = x - m
    v = jnp.mean(xc * xc, axis=-1, keepdims=True)
    return xc * lax.rsqrt(v + EPS)


def _gelu(x):
    inner = x * (GELU_C + (GELU_C * 0.044715) * (x * x))
    return (0.5 * x) * (1.0 + jnp.tanh(inner))


def _dot(a, b):
    return jnp.dot(a, b, preferred_element_type=F32)


def _pk(x):
    n = x.shape[0] // 16
    a = jnp.concatenate([x[16 * b:16 * b + 8] for b in range(n)], axis=0)
    b = jnp.concatenate([x[16 * b + 8:16 * b + 16] for b in range(n)], axis=0)
    return pltpu.pack_elementwise([a, b], packed_dtype=BF)


def _bf(x):
    return pltpu.bitcast(x, BF)


def _red8(x, op):
    parts = [x[8 * r:8 * r + 8] for r in range(x.shape[0] // 8)]
    while len(parts) > 1:
        parts = [op(parts[2 * r], parts[2 * r + 1]) for r in range(len(parts) // 2)] + (
            [parts[-1]] if len(parts) % 2 else [])
    return parts[0]


def _ln1_to(y_scr, x_v, row0, lo=0, hi=T):
    for c in range(lo // LNC, hi // LNC):
        x = x_v[pl.ds(row0 + c * LNC, LNC), :]
        y_scr[c * LNC:(c + 1) * LNC, :] = _ln(x.astype(F32)).astype(BF)


def _cp_x(x_hbm, x_v, sems, blk):
    rows = pl.ds(blk * T if isinstance(blk, int) else pl.multiple_of(blk * T, T), T)
    return pltpu.make_async_copy(x_hbm.at[rows, :], x_v.at[rows, :], sems.at[SEM_X + blk])


def _head_rhs(qT_blk):
    ws = []
    for h in range(4):
        pieces = []
        if h > 0:
            pieces.append(jnp.zeros((h * DH, QT), BF))
        pieces.append(qT_blk[h * DH:(h + 1) * DH])
        if h < 3:
            pieces.append(jnp.zeros(((3 - h) * DH, QT), BF))
        ws.append(jnp.concatenate(pieces, axis=0))
    return jnp.concatenate(ws, axis=1)


def _first_step(x_hbm, wqkv_hbm, wo_hbm, w1_hbm, b1_ref, w2_hbm, b2_ref, o_ref,
                x_v, wqkv_v, wo_v, w1_v, w2_v, k_scr, vt_scr, y_scr, raw_scr, qt_scr, ot_scr, acc_scr, sems):
    def col(c):
        return pl.ds(pl.multiple_of(c * WC, WC), WC)

    def cp_qkv(c):
        return pltpu.make_async_copy(wqkv_hbm.at[:, col(c)], wqkv_v.at[:, col(c)], sems.at[c])

    def cp_w1(c):
        return pltpu.make_async_copy(w1_hbm.at[:, col(c)], w1_v.at[:, col(c)], sems.at[SEM_W1 + c])

    def cp_w2(c):
        return pltpu.make_async_copy(w2_hbm.at[col(c), :], w2_v.at[col(c), :], sems.at[SEM_W2 + c])

    cp_wo = pltpu.make_async_copy(wo_hbm, wo_v, sems.at[SEM_WO])
    _cp_x(x_hbm, x_v, sems, 0).start()
    for c in range(NQKV):
        cp_qkv(c).start()
    _cp_x(x_hbm, x_v, sems, 1).start()
    cp_wo.start()
    for c in range(NFC):
        cp_w1(c).start()
        cp_w2(c).start()
    for blk in range(2, NSTEPS):
        _cp_x(x_hbm, x_v, sems, blk).start()

    _cp_x(x_hbm, x_v, sems, 0).wait()
    _ln1_to(y_scr, x_v, 0)

    def qkv_body(c, carry):
        cp_qkv(c).wait()
        scale = jnp.where(c < D // WC, QSCALE, 1.0).astype(F32)
        raw_scr[:, col(c)] = (_dot(y_scr[...], wqkv_v[:, col(c)]) * scale).astype(BF)
        return carry

    lax.fori_loop(0, NQKV, qkv_body, 0)

    qt_scr[...] = raw_scr[:, 0:D].T
    vT = _bf(_pk(raw_scr[:, 2 * D:3 * D].astype(F32))).T
    for jj in range(NQ):
        vt_scr[jj] = vT[:, jj * QT:(jj + 1) * QT]

    rr = lax.broadcasted_iota(jnp.int32, (QT, QT), 0)
    cc = lax.broadcasted_iota(jnp.int32, (QT, QT), 1)
    causal = rr <= cc

    def attn_scores(g):
        qT = qt_scr[pl.ds(pl.multiple_of(g * 128, 128), 128), :]
        kg = raw_scr[:, pl.ds(pl.multiple_of(D + g * 128, 128), 128)]
        return [_dot(kg[0:(j + 1) * QT], _head_rhs(qT[:, j * QT:(j + 1) * QT])) for j in range(NQ)]

    def attn_finish(g, scores):
        for j in range(NQ):
            for h in range(4):
                s = scores[j][:, h * QT:(h + 1) * QT]
                tiles = [s[t * QT:(t + 1) * QT] for t in range(j)] + [jnp.where(causal, s[j * QT:(j + 1) * QT], NEG)]
                m8 = _red8(tiles[0], jnp.maximum)
                for t in tiles[1:]:
                    m8 = jnp.maximum(m8, _red8(t, jnp.maximum))
                m = jnp.max(m8, axis=0, keepdims=True)
                es = [jnp.exp2(t - m) for t in tiles]
                l8 = _red8(es[0], jnp.add)
                for e in es[1:]:
                    l8 = l8 + _red8(e, jnp.add)
                l = jnp.sum(l8, axis=0, keepdims=True)
                rows = pl.ds(pl.multiple_of(g * 128 + h * DH, DH), DH)
                acc = _dot(vt_scr[0, rows, :], _bf(_pk(es[0])))
                for t in range(1, j + 1):
                    acc += _dot(vt_scr[t, rows, :], _bf(_pk(es[t])))
                ot_scr[rows, j * QT:(j + 1) * QT] = (acc * pl.reciprocal(l, approx=False)).astype(BF)

    def attn_body(gg, carry):
        scores = [attn_scores(gg * G0 + k) for k in range(G0)]
        for k in range(G0):
            attn_finish(gg * G0 + k, scores[k])
        return carry

    lax.fori_loop(0, NG // G0, attn_body, 0)

    cp_wo.wait()
    _cp_x(x_hbm, x_v, sems, 1).wait()
    k_scr[0:T, :] = raw_scr[:, D:2 * D]
    b2 = b2_ref[...].astype(F32).reshape(1, D)
    for j in range(NQ):
        attn = _dot(ot_scr[:, j * QT:(j + 1) * QT].T, wo_v[...])
        for c in range(QT // LNC):
            rows = slice(j * QT + c * LNC, j * QT + (c + 1) * LNC)
            hj = x_v[rows, :].astype(F32) + attn[c * LNC:(c + 1) * LNC]
            acc_scr[rows, :] = hj + b2
            raw_scr[rows, 0:D] = _ln(_ln(hj)).astype(BF)
    _ln1_to(y_scr, x_v, T, 0, YR)

    def mlp_body(c, carry):
        cp_w1(c).wait()
        cp_w2(c).wait()
        b1 = b1_ref[col(c)].astype(F32).reshape(1, WC)
        h = _gelu(_dot(raw_scr[:, 0:D], w1_v[:, col(c)]) + b1).astype(BF)
        acc_scr[...] += _dot(h, w2_v[col(c), :])
        return carry

    lax.fori_loop(0, NFC, mlp_body, 0)
    o_ref[...] = acc_scr[...].astype(o_ref.dtype)


def _main_step(i, b1_ref, b2_ref, o_ref, x_v, wqkv_v, wo_v, w1_v, w2_v, k_scr, vt_scr, y_scr):
    row0 = pl.multiple_of(i * T, T)
    rown = pl.multiple_of(jnp.minimum(i + 1, NSTEPS - 1) * T, T)
    ys = [_ln(x_v[pl.ds(row0 + c * LNC, LNC), :].astype(F32)).astype(BF) for c in range(YR // LNC, T // LNC)]
    qkv = jnp.concatenate([_dot(y_scr[0:YR, :], wqkv_v[...]), _dot(jnp.concatenate(ys, axis=0), wqkv_v[...])], axis=0)
    q32 = qkv[:, :D] * QSCALE
    k = qkv[:, D:2 * D].astype(BF)
    v = _bf(_pk(qkv[:, 2 * D:]))
    tbase = i * NQ
    k_scr[pl.ds(row0, T), :] = k
    even_d = (lax.broadcasted_iota(jnp.int32, (HQ, D), 1) // DH) % 2 == 0
    ra, rb = [], []
    for j in range(NQ):
        qa = q32[j * QT:j * QT + HQ]
        qb = q32[j * QT + HQ:(j + 1) * QT]
        ra.append(jnp.concatenate([jnp.where(even_d, qa, 0.0), jnp.where(even_d, 0.0, qa)], axis=0).astype(BF).T)
        rb.append(jnp.concatenate([jnp.where(even_d, 0.0, qb), jnp.where(even_d, qb, 0.0)], axis=0).astype(BF).T)
    vT = v.T
    for jj in range(NQ):
        vt_scr[tbase + jj] = vT[:, jj * QT:(jj + 1) * QT]

    rr = lax.broadcasted_iota(jnp.int32, (HQ, QT), 0)
    cc = lax.broadcasted_iota(jnp.int32, (HQ, QT), 1)
    lo64 = rr <= (cc % HQ)
    left1 = lax.broadcasted_iota(jnp.int32, (1, QT), 1) < HQ
    pr = lax.broadcasted_iota(jnp.int32, (HQ // 2, QT), 0)
    pc = lax.broadcasted_iota(jnp.int32, (HQ // 2, QT), 1)
    ca = (pr // 8) * 16 + pr % 8
    lo_bits = (jnp.where(ca <= pc % HQ, jnp.uint32(0x0000FFFF), jnp.uint32(0))
               | jnp.where(ca + 8 <= pc % HQ, jnp.uint32(0xFFFF0000), jnp.uint32(0)))
    hi_bits = ~lo_bits
    pleft = pc < HQ
    zero_u = jnp.zeros((HQ // 2, QT), jnp.uint32)
    left_hi = jnp.where(pleft, hi_bits, zero_u)
    left_lo = jnp.where(pleft, lo_bits, zero_u)
    right_hi = jnp.where(pleft, zero_u, hi_bits)
    right_lo = jnp.where(pleft, zero_u, lo_bits)
    pleft2 = lax.broadcasted_iota(jnp.int32, (HQ, QT), 1) < HQ

    def interleave(hi, lo):
        parts = []
        for b in range(HQ // 16):
            parts.append(hi[16 * b:16 * b + 16])
            parts.append(lo[16 * b:16 * b + 16])
        return parts

    def qk_operands(u):
        j, g = divmod(u, NG)
        start = pl.multiple_of((tbase + j - 2) * QT, QT)
        kwin = k_scr[pl.ds(start, 3 * QT), g * 128:(g + 1) * 128]
        blk = [kwin[HQ * b:HQ * (b + 1)] for b in range(6)]
        lhs_a = jnp.concatenate(interleave(blk[0], blk[4]) + [blk[1], blk[2], blk[3]], axis=0)
        lhs_b = jnp.concatenate(interleave(blk[1], blk[5]) + [blk[2], blk[3], blk[4]], axis=0)
        rhs = []
        for r in (ra[j], rb[j]):
            tiles = []
            for p in range(2):
                rows = r[g * 128 + 64 * p:g * 128 + 64 * (p + 1), :]
                z = jnp.zeros((64, QT), BF)
                tiles.append(jnp.concatenate([rows, z] if p == 0 else [z, rows], axis=0))
            rhs.append(jnp.concatenate(tiles, axis=1))
        return lhs_a, lhs_b, rhs[0], rhs[1]

    def qk_part(ops, p):
        lhs_a, lhs_b, rhs_a, rhs_b = ops
        sl = slice(p * PROWS, (p + 1) * PROWS)
        return _dot(lhs_a[sl], rhs_a), _dot(lhs_b[sl], rhs_b)

    def deinterleave(s):
        hi = jnp.concatenate([s[32 * b:32 * b + 16] for b in range(HQ // 16)], axis=0)
        lo = jnp.concatenate([s[32 * b + 16:32 * b + 32] for b in range(HQ // 16)], axis=0)
        return hi, lo

    def stage0(u, s_pair, p):
        j, g = divmod(u, NG)
        t0 = tbase + j - 2
        sa = s_pair[0][:, p * QT:(p + 1) * QT]
        sb = s_pair[1][:, p * QT:(p + 1) * QT]
        jg = tbase + j
        b2 = jnp.where(jg >= 2, 0.0, NEG).astype(F32)
        b1 = jnp.where(jg >= 1, 0.0, NEG).astype(F32)
        hi, lo = deinterleave(sa[0:2 * HQ])
        ma = jnp.where(lo64, lo, hi + b2)
        a3, a21 = sa[2 * HQ:3 * HQ], sa[3 * HQ:5 * HQ]
        m_a = jnp.max(jnp.maximum(jnp.maximum(_red8(ma, jnp.maximum), _red8(a3, jnp.maximum) + b2),
                                  _red8(a21, jnp.maximum) + b1), axis=0, keepdims=True)
        hi, lo = deinterleave(sb[0:2 * HQ])
        mb = jnp.where(lo64, lo, hi + b2)
        b21, b0 = sb[2 * HQ:4 * HQ], sb[4 * HQ:5 * HQ]
        m_b = jnp.max(jnp.maximum(jnp.maximum(_red8(mb, jnp.maximum), _red8(b0, jnp.maximum)),
                                  _red8(b21, jnp.maximum) + b1), axis=0, keepdims=True)
        e_a21 = jnp.exp2(a21 - (m_a - b1))
        e_b21 = jnp.exp2(b21 - (m_b - b1))
        l_a = _red8(e_a21, jnp.add)
        l_b = _red8(e_b21, jnp.add)
        r0 = g * 128 + 2 * p * DH
        pa, pb = _pk(e_a21), _pk(e_b21)
        acc_e = _dot(vt_scr[t0 + 1, r0:r0 + DH, :], _bf(jnp.where(pleft2, pa, pb)))
        acc_o = _dot(vt_scr[t0 + 1, r0 + DH:r0 + 2 * DH, :], _bf(jnp.where(pleft2, pb, pa)))
        return (ma, a3, m_a, l_a), (mb, b0, m_b, l_b), acc_e, acc_o

    def stage1(u, p, st):
        j, g = divmod(u, NG)
        t0 = tbase + j - 2
        (ma, a3, m_a, l_a), (mb, b0, m_b, l_b), acc_e, acc_o = st
        e_ma = jnp.exp2(ma - m_a)
        e_a3 = jnp.exp2(a3 - m_a)
        e_mb = jnp.exp2(mb - m_b)
        e_b0 = jnp.exp2(b0 - m_b)
        l_a = jnp.sum(l_a + _red8(e_ma + e_a3, jnp.add), axis=0, keepdims=True)
        l_b = jnp.sum(l_b + _red8(e_mb + e_b0, jnp.add), axis=0, keepdims=True)
        pma, pa3, pmb, pb0 = _pk(e_ma), _pk(e_a3), _pk(e_mb), _pk(e_b0)
        ma_lo = pma & lo_bits
        mb_hi = pmb & hi_bits
        r0 = g * 128 + 2 * p * DH
        pe0 = jnp.concatenate([pma & left_hi, jnp.where(pleft, pa3, mb_hi)], axis=0)
        pe2 = jnp.concatenate([jnp.where(pleft, ma_lo, pb0), pmb & right_lo], axis=0)
        po0 = jnp.concatenate([pma & right_hi, jnp.where(pleft, mb_hi, pa3)], axis=0)
        po2 = jnp.concatenate([jnp.where(pleft, pb0, ma_lo), pmb & left_lo], axis=0)
        acc_e += _dot(vt_scr[t0, r0:r0 + DH, :], _bf(pe0))
        acc_o += _dot(vt_scr[t0, r0 + DH:r0 + 2 * DH, :], _bf(po0))
        acc_e += _dot(vt_scr[t0 + 2, r0:r0 + DH, :], _bf(pe2))
        acc_o += _dot(vt_scr[t0 + 2, r0 + DH:r0 + 2 * DH, :], _bf(po2))
        r_a = pl.reciprocal(l_a, approx=False)
        r_b = pl.reciprocal(l_b, approx=False)
        o_e = acc_e * jnp.where(left1, r_a, r_b)
        o_o = pltpu.roll(acc_o * jnp.where(left1, r_b, r_a), HQ, 1)
        return o_e.astype(BF), o_o.astype(BF)

    NU = NQ * NG
    s_all = {}
    pair_p = {}
    head_out = {}

    def o_tile(j):
        oT = jnp.concatenate([head_out[4 * u + h] for u in range(j * NG, (j + 1) * NG) for h in range(4)], axis=0)
        return oT.T

    def gather(parts):
        return (jnp.concatenate([x[0] for x in parts], axis=0), jnp.concatenate([x[1] for x in parts], axis=0))

    ops = qk_operands(0)
    s_all[0] = gather([qk_part(ops, p) for p in range(NPART)])
    events = []
    for u in range(NU):
        ev = []
        for p in range(NPART):
            ev.append(((p + 0.0) / NPART, 0, "qk", u + 1, p))
        for st in range(4):
            ev.append(((st + LAGF) / 4.0, 1, "st", u, st))
        for pos, pri, kind, a_, b_ in ev:
            events.append((u + pos, pri, kind, a_, b_))
    events.sort(key=lambda e: (e[0], e[1]))
    nxt = {}
    attn0 = []
    o0 = None
    for _, _, kind, a_, b_ in events:
        if kind == "qk":
            un, p = a_, b_
            if un >= NU:
                if o0 is not None and len(attn0) < D // WOC:
                    c = len(attn0)
                    attn0.append(_dot(o0, wo_v[:, c * WOC:(c + 1) * WOC]))
                continue
            if p == 0:
                ops = qk_operands(un)
                nxt = []
            nxt.append(qk_part(ops, p))
            if p == NPART - 1:
                s_all[un] = gather(nxt)
                if un == NU - 1:
                    o0 = o_tile(0)
                    attn0.append(_dot(o0, wo_v[:, 0:WOC]))
        else:
            u, h = a_, b_
            hu = 4 * u + h
            if h % 2 == 0:
                pair_p[u] = stage0(u, s_all[u], h // 2)
            else:
                head_out[hu - 1], head_out[hu] = stage1(u, h // 2, pair_p[u])
    while len(attn0) < D // WOC:
        c = len(attn0)
        attn0.append(_dot(o0, wo_v[:, c * WOC:(c + 1) * WOC]))
    attn0 = jnp.concatenate(attn0, axis=1)

    hres = []

    def ln2(j, attn):
        ys = []
        for c in range(QT // LNC):
            r0 = j * QT + c * LNC
            hj = x_v[pl.ds(row0 + r0, LNC), :].astype(F32) + attn[c * LNC:(c + 1) * LNC]
            hres.append(hj)
            ys.append(_ln(_ln(hj)).astype(BF))
        return jnp.concatenate(ys, axis=0)

    b1 = b1_ref[...].astype(F32).reshape(1, F)
    y2a = ln2(0, attn0)
    attn1 = _dot(o_tile(1), wo_v[...])
    h1a0 = _gelu(_dot(y2a, w1_v[:, 0:FC0]) + b1[:, 0:FC0]).astype(BF)
    y2b = ln2(1, attn1)
    h1b0 = _gelu(_dot(y2b, w1_v[:, 0:FC0]) + b1[:, 0:FC0]).astype(BF)
    y2 = jnp.concatenate([y2a, y2b], axis=0)
    h1r = _gelu(_dot(y2, w1_v[:, FC0:]) + b1[:, FC0:]).astype(BF)
    h1a = jnp.concatenate([h1a0, h1r[0:QT]], axis=1)
    h1b = jnp.concatenate([h1b0, h1r[QT:]], axis=1)
    h1 = jnp.concatenate([h1a, h1b], axis=0)
    _ln1_to(y_scr, x_v, rown, 0, YR)
    out = _dot(h1, w2_v[...])
    hr = jnp.concatenate(hres, axis=0)
    o_ref[...] = (hr + out + b2_ref[...].astype(F32).reshape(1, D)).astype(o_ref.dtype)


def _kernel(x_hbm, wqkv_hbm, wo_hbm, w1_hbm, b1_ref, w2_hbm, b2_ref, o_ref,
            x_v, wqkv_v, wo_v, w1_v, w2_v, k_scr, vt_scr, y_scr, raw_scr, qt_scr, ot_scr, acc_scr, sems):
    i = pl.program_id(0)

    @pl.when(i == 0)
    def _():
        _first_step(x_hbm, wqkv_hbm, wo_hbm, w1_hbm, b1_ref, w2_hbm, b2_ref, o_ref,
                    x_v, wqkv_v, wo_v, w1_v, w2_v, k_scr, vt_scr, y_scr, raw_scr, qt_scr, ot_scr, acc_scr, sems)

    @pl.when(jnp.logical_and(i > 0, i + 1 < NSTEPS))
    def _():
        _cp_x(x_hbm, x_v, sems, i + 1).wait()

    @pl.when(i > 0)
    def _():
        _main_step(i, b1_ref, b2_ref, o_ref, x_v, wqkv_v, wo_v, w1_v, w2_v, k_scr, vt_scr, y_scr)


@jax.jit
def pallas_sequential_preLN__sliding_block__mixer_channel_mlp__prompt_kernel(A_x, A_wqkv, A_wo, B_x, B_w1, B_b1, B_w2, B_b2):
    x = A_x.reshape(S, D)
    out = pl.pallas_call(
        _kernel,
        grid=(NSTEPS,),
        in_specs=[
            pl.BlockSpec(memory_space=pl.ANY),
            pl.BlockSpec(memory_space=pl.ANY),
            pl.BlockSpec(memory_space=pl.ANY),
            pl.BlockSpec(memory_space=pl.ANY),
            pl.BlockSpec((F,), lambda i: (0,)),
            pl.BlockSpec(memory_space=pl.ANY),
            pl.BlockSpec((D,), lambda i: (0,)),
        ],
        out_specs=pl.BlockSpec((T, D), lambda i: (i, 0)),
        out_shape=jax.ShapeDtypeStruct((S, D), BF),
        scratch_shapes=[
            pltpu.VMEM((S, D), BF),
            pltpu.VMEM((D, 3 * D), BF),
            pltpu.VMEM((D, D), BF),
            pltpu.VMEM((D, F), BF),
            pltpu.VMEM((F, D), BF),
            pltpu.VMEM((S, D), BF),
            pltpu.VMEM((S // QT, D, QT), BF),
            pltpu.VMEM((T, D), BF),
            pltpu.VMEM((T, 3 * D), BF),
            pltpu.VMEM((D, T), BF),
            pltpu.VMEM((D, T), BF),
            pltpu.VMEM((T, D), F32),
            pltpu.SemaphoreType.DMA((NSEM,)),
        ],
        compiler_params=pltpu.CompilerParams(
            dimension_semantics=("arbitrary",),
            vmem_limit_bytes=100 * 1024 * 1024,
        ),
    )(x, A_wqkv, A_wo, B_w1, B_b1, B_w2, B_b2)
    return out.reshape(1, S, D)
```

```python
import jax
import jax.numpy as jnp
from jax import lax
import jax.experimental.pallas as pl
import jax.experimental.pallas.tpu as pltpu

S = 2048
D = 1024
F = 3584
DH = 32
T = 256
QT = 128
HQ = 64
NQ = T // QT
NSTEPS = S // T
NG = D // 128
EPS = 1e-5
NEG = -1e30
LOG2E = 1.4426950408889634
QSCALE = (DH ** -0.5) * LOG2E
GELU_C = 0.7978845608028654
BF = jnp.bfloat16
F32 = jnp.float32
NPART = 4
LNC = 16
KROWS = 5 * HQ
PROWS = KROWS // NPART
WOC = 128
LAGF = 1.75
YR = 128
FC0 = 512
WC = 512
NQKV = 3 * D // WC
NFC = F // WC
SEM_WO = NQKV
SEM_W1 = NQKV + 1
SEM_W2 = SEM_W1 + NFC
SEM_X = SEM_W2 + NFC
NSEM = SEM_X + S // T
G0 = 2


def _ln(x):
    m = jnp.mean(x, axis=-1, keepdims=True)
    xc = x - m
    v = jnp.mean(xc * xc, axis=-1, keepdims=True)
    return xc * lax.rsqrt(v + EPS)


def _gelu(x):
    inner = x * (GELU_C + (GELU_C * 0.044715) * (x * x))
    return (0.5 * x) * (1.0 + jnp.tanh(inner))


def _dot(a, b):
    return jnp.dot(a, b, preferred_element_type=F32)


def _pk(x):
    n = x.shape[0] // 16
    a = jnp.concatenate([x[16 * b:16 * b + 8] for b in range(n)], axis=0)
    b = jnp.concatenate([x[16 * b + 8:16 * b + 16] for b in range(n)], axis=0)
    return pltpu.pack_elementwise([a, b], packed_dtype=BF)


def _bf(x):
    return pltpu.bitcast(x, BF)


def _red8(x, op):
    parts = [x[8 * r:8 * r + 8] for r in range(x.shape[0] // 8)]
    while len(parts) > 1:
        parts = [op(parts[2 * r], parts[2 * r + 1]) for r in range(len(parts) // 2)] + (
            [parts[-1]] if len(parts) % 2 else [])
    return parts[0]


def _ln1_to(y_scr, x_v, row0, lo=0, hi=T):
    for c in range(lo // LNC, hi // LNC):
        x = x_v[pl.ds(row0 + c * LNC, LNC), :]
        y_scr[c * LNC:(c + 1) * LNC, :] = _ln(x.astype(F32)).astype(BF)


def _cp_x(x_hbm, x_v, sems, blk):
    rows = pl.ds(blk * T if isinstance(blk, int) else pl.multiple_of(blk * T, T), T)
    return pltpu.make_async_copy(x_hbm.at[rows, :], x_v.at[rows, :], sems.at[SEM_X + blk])


def _head_rhs(qT_blk):
    ws = []
    for h in range(4):
        pieces = []
        if h > 0:
            pieces.append(jnp.zeros((h * DH, QT), BF))
        pieces.append(qT_blk[h * DH:(h + 1) * DH])
        if h < 3:
            pieces.append(jnp.zeros(((3 - h) * DH, QT), BF))
        ws.append(jnp.concatenate(pieces, axis=0))
    return jnp.concatenate(ws, axis=1)


def _first_step(x_hbm, wqkv_hbm, wo_hbm, w1_hbm, b1_ref, w2_hbm, b2_ref, o_ref,
                x_v, wqkv_v, wo_v, w1_v, w2_v, k_scr, vt_scr, y_scr, raw_scr, qt_scr, ot_scr, acc_scr, sems):
    def col(c):
        return pl.ds(pl.multiple_of(c * WC, WC), WC)

    def cp_qkv(c):
        return pltpu.make_async_copy(wqkv_hbm.at[:, col(c)], wqkv_v.at[:, col(c)], sems.at[c])

    def cp_w1(c):
        return pltpu.make_async_copy(w1_hbm.at[:, col(c)], w1_v.at[:, col(c)], sems.at[SEM_W1 + c])

    def cp_w2(c):
        return pltpu.make_async_copy(w2_hbm.at[col(c), :], w2_v.at[col(c), :], sems.at[SEM_W2 + c])

    cp_wo = pltpu.make_async_copy(wo_hbm, wo_v, sems.at[SEM_WO])
    _cp_x(x_hbm, x_v, sems, 0).start()
    for c in range(NQKV):
        cp_qkv((c + 4) % NQKV).start()
    _cp_x(x_hbm, x_v, sems, 1).start()
    cp_wo.start()
    for c in range(NFC):
        cp_w1(c).start()
        cp_w2(c).start()
    for blk in range(2, NSTEPS):
        _cp_x(x_hbm, x_v, sems, blk).start()

    _cp_x(x_hbm, x_v, sems, 0).wait()
    _ln1_to(y_scr, x_v, 0)

    def qkv_chunk(cid):
        cp_qkv(cid).wait()
        scale = jnp.where(cid < D // WC, QSCALE, 1.0).astype(F32)
        raw_scr[:, col(cid)] = (_dot(y_scr[...], wqkv_v[:, col(cid)]) * scale).astype(BF)

    def qkv_body(c, carry):
        qkv_chunk(lax.rem(c + 4, NQKV))
        return carry

    lax.fori_loop(0, NQKV - 1, qkv_body, 0)
    qkv_chunk((NQKV - 1 + 4) % NQKV)

    qt_scr[...] = raw_scr[:, 0:D].T
    vT = _bf(_pk(raw_scr[:, 2 * D:3 * D].astype(F32))).T
    for jj in range(NQ):
        vt_scr[jj] = vT[:, jj * QT:(jj + 1) * QT]

    rr = lax.broadcasted_iota(jnp.int32, (QT, QT), 0)
    cc = lax.broadcasted_iota(jnp.int32, (QT, QT), 1)
    causal = rr <= cc

    def attn_scores(g):
        qT = qt_scr[pl.ds(pl.multiple_of(g * 128, 128), 128), :]
        kg = raw_scr[:, pl.ds(pl.multiple_of(D + g * 128, 128), 128)]
        return [_dot(kg[0:(j + 1) * QT], _head_rhs(qT[:, j * QT:(j + 1) * QT])) for j in range(NQ)]

    def attn_finish(g, scores):
        for j in range(NQ):
            for h in range(4):
                s = scores[j][:, h * QT:(h + 1) * QT]
                tiles = [s[t * QT:(t + 1) * QT] for t in range(j)] + [jnp.where(causal, s[j * QT:(j + 1) * QT], NEG)]
                m8 = _red8(tiles[0], jnp.maximum)
                for t in tiles[1:]:
                    m8 = jnp.maximum(m8, _red8(t, jnp.maximum))
                m = jnp.max(m8, axis=0, keepdims=True)
                es = [jnp.exp2(t - m) for t in tiles]
                l8 = _red8(es[0], jnp.add)
                for e in es[1:]:
                    l8 = l8 + _red8(e, jnp.add)
                l = jnp.sum(l8, axis=0, keepdims=True)
                rows = pl.ds(pl.multiple_of(g * 128 + h * DH, DH), DH)
                acc = _dot(vt_scr[0, rows, :], _bf(_pk(es[0])))
                for t in range(1, j + 1):
                    acc += _dot(vt_scr[t, rows, :], _bf(_pk(es[t])))
                ot_scr[rows, j * QT:(j + 1) * QT] = (acc * pl.reciprocal(l, approx=False)).astype(BF)

    def attn_body(gg, carry):
        scores = [attn_scores(gg * G0 + k) for k in range(G0)]
        for k in range(G0):
            attn_finish(gg * G0 + k, scores[k])
        return carry

    lax.fori_loop(0, NG // G0, attn_body, 0)

    cp_wo.wait()
    _cp_x(x_hbm, x_v, sems, 1).wait()
    k_scr[0:T, :] = raw_scr[:, D:2 * D]
    b2 = b2_ref[...].astype(F32).reshape(1, D)
    for j in range(NQ):
        attn = _dot(ot_scr[:, j * QT:(j + 1) * QT].T, wo_v[...])
        for c in range(QT // LNC):
            rows = slice(j * QT + c * LNC, j * QT + (c + 1) * LNC)
            hj = x_v[rows, :].astype(F32) + attn[c * LNC:(c + 1) * LNC]
            acc_scr[rows, :] = hj + b2
            raw_scr[rows, 0:D] = _ln(_ln(hj)).astype(BF)
    _ln1_to(y_scr, x_v, T, 0, YR)

    def mlp_body(c, carry):
        cp_w1(c).wait()
        cp_w2(c).wait()
        b1 = b1_ref[col(c)].astype(F32).reshape(1, WC)
        h = _gelu(_dot(raw_scr[:, 0:D], w1_v[:, col(c)]) + b1).astype(BF)
        acc_scr[...] += _dot(h, w2_v[col(c), :])
        return carry

    lax.fori_loop(0, NFC, mlp_body, 0)
    o_ref[...] = acc_scr[...].astype(o_ref.dtype)


def _main_step(i, b1_ref, b2_ref, o_ref, x_v, wqkv_v, wo_v, w1_v, w2_v, k_scr, vt_scr, y_scr):
    row0 = pl.multiple_of(i * T, T)
    rown = pl.multiple_of(jnp.minimum(i + 1, NSTEPS - 1) * T, T)
    ys = [_ln(x_v[pl.ds(row0 + c * LNC, LNC), :].astype(F32)).astype(BF) for c in range(YR // LNC, T // LNC)]
    qkv = jnp.concatenate([_dot(y_scr[0:YR, :], wqkv_v[...]), _dot(jnp.concatenate(ys, axis=0), wqkv_v[...])], axis=0)
    q32 = qkv[:, :D] * QSCALE
    k = qkv[:, D:2 * D].astype(BF)
    v = _bf(_pk(qkv[:, 2 * D:]))
    tbase = i * NQ
    k_scr[pl.ds(row0, T), :] = k
    even_d = (lax.broadcasted_iota(jnp.int32, (HQ, D), 1) // DH) % 2 == 0
    ra, rb = [], []
    for j in range(NQ):
        qa = q32[j * QT:j * QT + HQ]
        qb = q32[j * QT + HQ:(j + 1) * QT]
        ra.append(jnp.concatenate([jnp.where(even_d, qa, 0.0), jnp.where(even_d, 0.0, qa)], axis=0).astype(BF).T)
        rb.append(jnp.concatenate([jnp.where(even_d, 0.0, qb), jnp.where(even_d, qb, 0.0)], axis=0).astype(BF).T)
    vT = v.T
    for jj in range(NQ):
        vt_scr[tbase + jj] = vT[:, jj * QT:(jj + 1) * QT]

    rr = lax.broadcasted_iota(jnp.int32, (HQ, QT), 0)
    cc = lax.broadcasted_iota(jnp.int32, (HQ, QT), 1)
    lo64 = rr <= (cc % HQ)
    left1 = lax.broadcasted_iota(jnp.int32, (1, QT), 1) < HQ
    pr = lax.broadcasted_iota(jnp.int32, (HQ // 2, QT), 0)
    pc = lax.broadcasted_iota(jnp.int32, (HQ // 2, QT), 1)
    ca = (pr // 8) * 16 + pr % 8
    lo_bits = (jnp.where(ca <= pc % HQ, jnp.uint32(0x0000FFFF), jnp.uint32(0))
               | jnp.where(ca + 8 <= pc % HQ, jnp.uint32(0xFFFF0000), jnp.uint32(0)))
    hi_bits = ~lo_bits
    pleft = pc < HQ
    zero_u = jnp.zeros((HQ // 2, QT), jnp.uint32)
    left_hi = jnp.where(pleft, hi_bits, zero_u)
    left_lo = jnp.where(pleft, lo_bits, zero_u)
    right_hi = jnp.where(pleft, zero_u, hi_bits)
    right_lo = jnp.where(pleft, zero_u, lo_bits)
    pleft2 = lax.broadcasted_iota(jnp.int32, (HQ, QT), 1) < HQ

    def interleave(hi, lo):
        parts = []
        for b in range(HQ // 16):
            parts.append(hi[16 * b:16 * b + 16])
            parts.append(lo[16 * b:16 * b + 16])
        return parts

    def qk_operands(u):
        j, g = divmod(u, NG)
        start = pl.multiple_of((tbase + j - 2) * QT, QT)
        kwin = k_scr[pl.ds(start, 3 * QT), g * 128:(g + 1) * 128]
        blk = [kwin[HQ * b:HQ * (b + 1)] for b in range(6)]
        lhs_a = jnp.concatenate(interleave(blk[0], blk[4]) + [blk[1], blk[2], blk[3]], axis=0)
        lhs_b = jnp.concatenate(interleave(blk[1], blk[5]) + [blk[2], blk[3], blk[4]], axis=0)
        rhs = []
        for r in (ra[j], rb[j]):
            tiles = []
            for p in range(2):
                rows = r[g * 128 + 64 * p:g * 128 + 64 * (p + 1), :]
                z = jnp.zeros((64, QT), BF)
                tiles.append(jnp.concatenate([rows, z] if p == 0 else [z, rows], axis=0))
            rhs.append(jnp.concatenate(tiles, axis=1))
        return lhs_a, lhs_b, rhs[0], rhs[1]

    def qk_part(ops, p):
        lhs_a, lhs_b, rhs_a, rhs_b = ops
        sl = slice(p * PROWS, (p + 1) * PROWS)
        return _dot(lhs_a[sl], rhs_a), _dot(lhs_b[sl], rhs_b)

    def deinterleave(s):
        hi = jnp.concatenate([s[32 * b:32 * b + 16] for b in range(HQ // 16)], axis=0)
        lo = jnp.concatenate([s[32 * b + 16:32 * b + 32] for b in range(HQ // 16)], axis=0)
        return hi, lo

    def stage0(u, s_pair, p):
        j, g = divmod(u, NG)
        t0 = tbase + j - 2
        sa = s_pair[0][:, p * QT:(p + 1) * QT]
        sb = s_pair[1][:, p * QT:(p + 1) * QT]
        jg = tbase + j
        b2 = jnp.where(jg >= 2, 0.0, NEG).astype(F32)
        b1 = jnp.where(jg >= 1, 0.0, NEG).astype(F32)
        hi, lo = deinterleave(sa[0:2 * HQ])
        ma = jnp.where(lo64, lo, hi + b2)
        a3, a21 = sa[2 * HQ:3 * HQ], sa[3 * HQ:5 * HQ]
        m_a = jnp.max(jnp.maximum(jnp.maximum(_red8(ma, jnp.maximum), _red8(a3, jnp.maximum) + b2),
                                  _red8(a21, jnp.maximum) + b1), axis=0, keepdims=True)
        hi, lo = deinterleave(sb[0:2 * HQ])
        mb = jnp.where(lo64, lo, hi + b2)
        b21, b0 = sb[2 * HQ:4 * HQ], sb[4 * HQ:5 * HQ]
        m_b = jnp.max(jnp.maximum(jnp.maximum(_red8(mb, jnp.maximum), _red8(b0, jnp.maximum)),
                                  _red8(b21, jnp.maximum) + b1), axis=0, keepdims=True)
        e_a21 = jnp.exp2(a21 - (m_a - b1))
        e_b21 = jnp.exp2(b21 - (m_b - b1))
        l_a = _red8(e_a21, jnp.add)
        l_b = _red8(e_b21, jnp.add)
        r0 = g * 128 + 2 * p * DH
        pa, pb = _pk(e_a21), _pk(e_b21)
        acc_e = _dot(vt_scr[t0 + 1, r0:r0 + DH, :], _bf(jnp.where(pleft2, pa, pb)))
        acc_o = _dot(vt_scr[t0 + 1, r0 + DH:r0 + 2 * DH, :], _bf(jnp.where(pleft2, pb, pa)))
        return (ma, a3, m_a, l_a), (mb, b0, m_b, l_b), acc_e, acc_o

    def stage1(u, p, st):
        j, g = divmod(u, NG)
        t0 = tbase + j - 2
        (ma, a3, m_a, l_a), (mb, b0, m_b, l_b), acc_e, acc_o = st
        e_ma = jnp.exp2(ma - m_a)
        e_a3 = jnp.exp2(a3 - m_a)
        e_mb = jnp.exp2(mb - m_b)
        e_b0 = jnp.exp2(b0 - m_b)
        l_a = jnp.sum(l_a + _red8(e_ma + e_a3, jnp.add), axis=0, keepdims=True)
        l_b = jnp.sum(l_b + _red8(e_mb + e_b0, jnp.add), axis=0, keepdims=True)
        pma, pa3, pmb, pb0 = _pk(e_ma), _pk(e_a3), _pk(e_mb), _pk(e_b0)
        ma_lo = pma & lo_bits
        mb_hi = pmb & hi_bits
        r0 = g * 128 + 2 * p * DH
        pe0 = jnp.concatenate([pma & left_hi, jnp.where(pleft, pa3, mb_hi)], axis=0)
        pe2 = jnp.concatenate([jnp.where(pleft, ma_lo, pb0), pmb & right_lo], axis=0)
        po0 = jnp.concatenate([pma & right_hi, jnp.where(pleft, mb_hi, pa3)], axis=0)
        po2 = jnp.concatenate([jnp.where(pleft, pb0, ma_lo), pmb & left_lo], axis=0)
        acc_e += _dot(vt_scr[t0, r0:r0 + DH, :], _bf(pe0))
        acc_o += _dot(vt_scr[t0, r0 + DH:r0 + 2 * DH, :], _bf(po0))
        acc_e += _dot(vt_scr[t0 + 2, r0:r0 + DH, :], _bf(pe2))
        acc_o += _dot(vt_scr[t0 + 2, r0 + DH:r0 + 2 * DH, :], _bf(po2))
        r_a = pl.reciprocal(l_a, approx=False)
        r_b = pl.reciprocal(l_b, approx=False)
        o_e = acc_e * jnp.where(left1, r_a, r_b)
        o_o = pltpu.roll(acc_o * jnp.where(left1, r_b, r_a), HQ, 1)
        return o_e.astype(BF), o_o.astype(BF)

    NU = NQ * NG
    s_all = {}
    pair_p = {}
    head_out = {}

    def o_tile(j):
        oT = jnp.concatenate([head_out[4 * u + h] for u in range(j * NG, (j + 1) * NG) for h in range(4)], axis=0)
        return oT.T

    def gather(parts):
        return (jnp.concatenate([x[0] for x in parts], axis=0), jnp.concatenate([x[1] for x in parts], axis=0))

    ops = qk_operands(0)
    s_all[0] = gather([qk_part(ops, p) for p in range(NPART)])
    events = []
    for u in range(NU):
        ev = []
        for p in range(NPART):
            ev.append(((p + 0.0) / NPART, 0, "qk", u + 1, p))
        for st in range(4):
            ev.append(((st + LAGF) / 4.0, 1, "st", u, st))
        for pos, pri, kind, a_, b_ in ev:
            events.append((u + pos, pri, kind, a_, b_))
    events.sort(key=lambda e: (e[0], e[1]))
    nxt = {}
    attn0 = []
    o0 = None
    for _, _, kind, a_, b_ in events:
        if kind == "qk":
            un, p = a_, b_
            if un >= NU:
                if o0 is not None and len(attn0) < D // WOC:
                    c = len(attn0)
                    attn0.append(_dot(o0, wo_v[:, c * WOC:(c + 1) * WOC]))
                continue
            if p == 0:
                ops = qk_operands(un)
                nxt = []
            nxt.append(qk_part(ops, p))
            if p == NPART - 1:
                s_all[un] = gather(nxt)
                if un == NU - 1:
                    o0 = o_tile(0)
                    attn0.append(_dot(o0, wo_v[:, 0:WOC]))
        else:
            u, h = a_, b_
            hu = 4 * u + h
            if h % 2 == 0:
                pair_p[u] = stage0(u, s_all[u], h // 2)
            else:
                head_out[hu - 1], head_out[hu] = stage1(u, h // 2, pair_p[u])
    while len(attn0) < D // WOC:
        c = len(attn0)
        attn0.append(_dot(o0, wo_v[:, c * WOC:(c + 1) * WOC]))
    attn0 = jnp.concatenate(attn0, axis=1)

    hres = []

    def ln2(j, attn):
        ys = []
        for c in range(QT // LNC):
            r0 = j * QT + c * LNC
            hj = x_v[pl.ds(row0 + r0, LNC), :].astype(F32) + attn[c * LNC:(c + 1) * LNC]
            hres.append(hj)
            ys.append(_ln(_ln(hj)).astype(BF))
        return jnp.concatenate(ys, axis=0)

    b1 = b1_ref[...].astype(F32).reshape(1, F)
    y2a = ln2(0, attn0)
    attn1 = _dot(o_tile(1), wo_v[...])
    h1a0 = _gelu(_dot(y2a, w1_v[:, 0:FC0]) + b1[:, 0:FC0]).astype(BF)
    y2b = ln2(1, attn1)
    h1b0 = jnp.concatenate([_gelu(_dot(y2b[r:r + HQ], w1_v[:, 0:FC0]) + b1[:, 0:FC0]).astype(BF)
                            for r in range(0, QT, HQ)], axis=0)
    y2 = jnp.concatenate([y2a, y2b], axis=0)
    h1r = _gelu(_dot(y2, w1_v[:, FC0:]) + b1[:, FC0:]).astype(BF)
    h1a = jnp.concatenate([h1a0, h1r[0:QT]], axis=1)
    h1b = jnp.concatenate([h1b0, h1r[QT:]], axis=1)
    h1 = jnp.concatenate([h1a, h1b], axis=0)
    _ln1_to(y_scr, x_v, rown, 0, YR)
    out = _dot(h1, w2_v[...])
    hr = jnp.concatenate(hres, axis=0)
    o_ref[...] = (hr + out + b2_ref[...].astype(F32).reshape(1, D)).astype(o_ref.dtype)


def _kernel(x_hbm, wqkv_hbm, wo_hbm, w1_hbm, b1_ref, w2_hbm, b2_ref, o_ref,
            x_v, wqkv_v, wo_v, w1_v, w2_v, k_scr, vt_scr, y_scr, raw_scr, qt_scr, ot_scr, acc_scr, sems):
    i = pl.program_id(0)

    @pl.when(i == 0)
    def _():
        _first_step(x_hbm, wqkv_hbm, wo_hbm, w1_hbm, b1_ref, w2_hbm, b2_ref, o_ref,
                    x_v, wqkv_v, wo_v, w1_v, w2_v, k_scr, vt_scr, y_scr, raw_scr, qt_scr, ot_scr, acc_scr, sems)

    @pl.when(jnp.logical_and(i > 0, i + 1 < NSTEPS))
    def _():
        _cp_x(x_hbm, x_v, sems, i + 1).wait()

    @pl.when(i > 0)
    def _():
        _main_step(i, b1_ref, b2_ref, o_ref, x_v, wqkv_v, wo_v, w1_v, w2_v, k_scr, vt_scr, y_scr)


@jax.jit
def pallas_sequential_preLN__sliding_block__mixer_channel_mlp__prompt_kernel(A_x, A_wqkv, A_wo, B_x, B_w1, B_b1, B_w2, B_b2):
    x = A_x.reshape(S, D)
    out = pl.pallas_call(
        _kernel,
        grid=(NSTEPS,),
        in_specs=[
            pl.BlockSpec(memory_space=pl.ANY),
            pl.BlockSpec(memory_space=pl.ANY),
            pl.BlockSpec(memory_space=pl.ANY),
            pl.BlockSpec(memory_space=pl.ANY),
            pl.BlockSpec((F,), lambda i: (0,)),
            pl.BlockSpec(memory_space=pl.ANY),
            pl.BlockSpec((D,), lambda i: (0,)),
        ],
        out_specs=pl.BlockSpec((T, D), lambda i: (i, 0)),
        out_shape=jax.ShapeDtypeStruct((S, D), BF),
        scratch_shapes=[
            pltpu.VMEM((S, D), BF),
            pltpu.VMEM((D, 3 * D), BF),
            pltpu.VMEM((D, D), BF),
            pltpu.VMEM((D, F), BF),
            pltpu.VMEM((F, D), BF),
            pltpu.VMEM((S, D), BF),
            pltpu.VMEM((S // QT, D, QT), BF),
            pltpu.VMEM((T, D), BF),
            pltpu.VMEM((T, 3 * D), BF),
            pltpu.VMEM((D, T), BF),
            pltpu.VMEM((D, T), BF),
            pltpu.VMEM((T, D), F32),
            pltpu.SemaphoreType.DMA((NSEM,)),
        ],
        compiler_params=pltpu.CompilerParams(
            dimension_semantics=("arbitrary",),
            vmem_limit_bytes=100 * 1024 * 1024,
        ),
    )(x, A_wqkv, A_wo, B_w1, B_b1, B_w2, B_b2)
    return out.reshape(1, S, D)
```
